```python
import jax
import jax.numpy as jnp

def _softmax(x, axis=-1):
    return jax.nn.softmax(x, axis=axis)
def _gelu(x):
    return jax.nn.gelu(x, approximate=True)
def _silu(x):
    return jax.nn.silu(x)
def _sigmoid(x):
    return jax.nn.sigmoid(x)
def _layernorm(x, axis=-1, eps=1e-5):
    m = jnp.mean(x, axis=axis, keepdims=True)
    v = jnp.var(x, axis=axis, keepdims=True)
    return (x - m) / jnp.sqrt(v + eps)
def _scatter_add(tgt, idx, src, axis=0):
    return tgt.at[idx].add(src)
def _segment_sum(src, seg, n):
    return jax.ops.segment_sum(src, seg, n)
class _Rng:
    def __init__(self, key):
        self._k = key
    def _next(self):
        self._k, sub = jax.random.split(self._k)
        return sub
    def normal(self, shape):
        return jax.random.normal(self._next(), shape, dtype=jnp.bfloat16)
    def randint(self, lo, hi, shape):
        return jax.random.randint(self._next(), shape, lo, hi, dtype=jnp.int32)
    def uniform(self, shape, lo=0.0, hi=1.0):
        return jax.random.uniform(self._next(), shape, jnp.bfloat16, lo, hi)
    def permutation(self, n):
        return jax.random.permutation(self._next(), n)


kernel_name = 'parallel_sum__sliding_block_cached__glu_gated_swiglu__decode'

def setup_inputs():
    _rng = _Rng(jax.random.key(int.from_bytes(__import__("os").urandom(4), "little")))
    _w = (lambda a: (lambda t: t.astype(jnp.bfloat16) if jnp.issubdtype(t.dtype, jnp.floating) else t)(jnp.asarray(a)))
    def _A_setup():
        B, Sq, D = 4, 1, 640
        Hq, Hkv, Sk, Dh = 32, 32, 8192, 192
        assert Hq % Hkv == 0, (Hq, Hkv)
        return {
            "x": _w((lambda *s: _rng.normal(s) * 0.05)(B, Sq, D)),
            "k_cache": _w((lambda *s: _rng.normal(s) * 0.05)(B, Hkv, Sk, Dh)),
            "v_cache": _w((lambda *s: _rng.normal(s) * 0.05)(B, Hkv, Sk, Dh)),
            "wq": _w((lambda *s: _rng.normal(s) * 0.05)(D, Hq * Dh) * (D ** -0.5)),
            "wo": _w((lambda *s: _rng.normal(s) * 0.05)(Hq * Dh, D) * ((Hq * Dh) ** -0.5)),
        }
    _A_in = _A_setup()

    def _B_setup():
        B, S, D, F = 4, 1, 640, 1536
        return {
            "x": _w((lambda *s: _rng.normal(s) * 0.05)(B, S, D)),
            "w1": _w((lambda *s: _rng.normal(s) * 0.05)(D, F) * (2.0 / D) ** 0.5),
            "w3": _w((lambda *s: _rng.normal(s) * 0.05)(D, F) * (2.0 / D) ** 0.5),
            "w2": _w((lambda *s: _rng.normal(s) * 0.05)(F, D) * (2.0 / F) ** 0.5),
        }
    _B_in = _B_setup()

    return {
        "A_x": _A_in["x"],
        "A_k_cache": _A_in["k_cache"],
        "A_v_cache": _A_in["v_cache"],
        "A_wq": _A_in["wq"],
        "A_wo": _A_in["wo"],
        "B_x": _B_in["x"],
        "B_w1": _B_in["w1"],
        "B_w3": _B_in["w3"],
        "B_w2": _B_in["w2"],
    }

def reference(A_x, A_k_cache, A_v_cache, A_wq, A_wo, B_x, B_w1, B_w3, B_w2):
    def _A_ref(x, k_cache, v_cache, wq, wo):
        B, Sq, D = x.shape
        Hq, Dh = 32, 192
        Hkv, Sk = k_cache.shape[1], k_cache.shape[2]
        W = min(4096, max(256, Sk // 4))
        rep = Hq // Hkv
        q = (lambda x, *d: x.transpose(*d))((x @ wq).reshape(B, Sq, Hq, Dh), 0, 2, 1, 3)
        k = jnp.repeat(k_cache[:, :, Sk - W:, :], rep, axis=1)
        v = jnp.repeat(v_cache[:, :, Sk - W:, :], rep, axis=1)
        scores = jnp.einsum("bhqd,bhkd->bhqk", q, k) * (Dh ** -0.5)
        p = _softmax(scores, axis=-1)
        o = jnp.einsum("bhqk,bhkd->bhqd", p, v)
        return (lambda x, *d: x.transpose(*d))(o, 0, 2, 1, 3).reshape(B, Sq, Hq * Dh) @ wo

    def _B_ref(x, w1, w3, w2):
        gate = jnp.einsum("bsd,df->bsf", x, w1)
        up = jnp.einsum("bsd,df->bsf", x, w3)
        h = _silu(gate) * up
        out = jnp.einsum("bsf,fd->bsd", h, w2)
        return out

    x = A_x
    xn = _layernorm(x, axis=-1)
    return x + _A_ref(xn, A_k_cache, A_v_cache, A_wq, A_wo) + _B_ref(xn, B_w1, B_w3, B_w2)
```

```python
import jax
import jax.numpy as jnp
from jax import lax
import jax.experimental.pallas as pl
import jax.experimental.pallas.tpu as pltpu

HG = 8
NBUF = 3
NW2 = 4
LN_EPS = 1e-5


@jax.jit
def pallas_parallel_sum__sliding_block_cached__glu_gated_swiglu__decode_kernel(
    A_x: jax.Array,
    A_k_cache: jax.Array,
    A_v_cache: jax.Array,
    A_wq: jax.Array,
    A_wo: jax.Array,
    B_x: jax.Array,
    B_w1: jax.Array,
    B_w3: jax.Array,
    B_w2: jax.Array,
):
    del B_x
    B, Sq, D = A_x.shape
    _, H, Sk, Dh = A_k_cache.shape
    F = B_w1.shape[1]
    assert Sq == 1 and B <= 8 and H % HG == 0 and A_wq.shape == (D, H * Dh)
    W = min(4096, max(256, Sk // 4))
    NG = H // HG
    GR = HG * Dh
    NSTEP = NG * B
    FC = F // NW2
    scale = Dh ** -0.5
    f32, bf16 = jnp.float32, jnp.bfloat16
    dt = A_x.dtype

    def kernel_function(x_hbm, kt_hbm, vt_hbm, wq_hbm, wo_hbm, w1_hbm, w3_hbm, w2_hbm,
                        out_ref,
                        x_v, wq_v, wo_v, w1_v, w3_v, w2_v, kbuf, vbuf, q_v, o_v,
                        sem_w, sem_wo, sem_w2, sem_k, sem_v):

        def kv_copy(src, dst, sem, step):
            g, b = step // B, step % B
            row = (b * NG + g) * GR
            slot = step % NBUF
            if not isinstance(step, int):
                row = pl.multiple_of(row, GR)
            return pltpu.make_async_copy(
                src.at[pl.ds(row, GR), pl.ds(Sk - W, W)], dst.at[slot], sem.at[slot])

        def k_copy(step):
            return kv_copy(kt_hbm, kbuf, sem_k, step)

        def v_copy(step):
            return kv_copy(vt_hbm, vbuf, sem_v, step)

        def wo_copy(g):
            return pltpu.make_async_copy(
                wo_hbm.at[pl.ds(g * GR, GR)], wo_v.at[pl.ds(g * GR, GR)], sem_wo.at[g])

        def w2_copy(c):
            return pltpu.make_async_copy(
                w2_hbm.at[pl.ds(c * FC, FC)], w2_v.at[pl.ds(c * FC, FC)], sem_w2.at[c])

        x_cp = pltpu.make_async_copy(x_hbm, x_v, sem_w.at[0])
        wq_cp = pltpu.make_async_copy(wq_hbm, wq_v, sem_w.at[1])
        w1_cp = pltpu.make_async_copy(w1_hbm, w1_v, sem_w.at[2])
        w3_cp = pltpu.make_async_copy(w3_hbm, w3_v, sem_w.at[3])

        wq_cp.start()
        x_cp.start()
        for s in range(NBUF):
            k_copy(s).start()
            v_copy(s).start()

        x_cp.wait()
        x = x_v[...].astype(f32)
        mean = jnp.mean(x, axis=-1, keepdims=True)
        xc = x - mean
        var = jnp.mean(xc * xc, axis=-1, keepdims=True)
        xn = (xc / jnp.sqrt(var + LN_EPS)).astype(dt)

        wq_cp.wait()
        q = jnp.dot(xn, wq_v[...], preferred_element_type=f32)
        q_v[...] = q.astype(dt).astype(f32)

        col = lax.broadcasted_iota(jnp.int32, (HG, GR), 1)
        lo = lax.broadcasted_iota(jnp.int32, (HG, GR), 0) * Dh
        diag = jnp.logical_and(col >= lo, col < lo + Dh)

        def attn_step(step, g, b):
            slot = step % NBUF
            qrow = q_v[pl.ds(b, 1), pl.ds(g * GR, GR)]
            qd = jnp.where(diag, jnp.broadcast_to(qrow, (HG, GR)), 0.0).astype(dt)
            k_copy(step).wait()
            s = jnp.dot(qd, kbuf[slot], preferred_element_type=f32) * scale

            @pl.when(step + NBUF < NSTEP)
            def _():
                k_copy(step + NBUF).start()

            m = jnp.max(s, axis=-1, keepdims=True)
            e = jnp.exp(s - m)
            p = (e / jnp.sum(e, axis=-1, keepdims=True)).astype(dt)
            v_copy(step).wait()
            o = lax.dot_general(p, vbuf[slot], (((1,), (1,)), ((), ())),
                                preferred_element_type=f32)

            @pl.when(step + NBUF < NSTEP)
            def _():
                v_copy(step + NBUF).start()

            o_v[pl.ds(b, 1), :] = jnp.sum(jnp.where(diag, o, 0.0), axis=0, keepdims=True)

        acc = jnp.zeros((B, D), f32)
        h = None
        for g in range(NG):
            wo_copy(g).start()
            if g == 0:
                w1_cp.start()
            if g == 1:
                w3_cp.start()
            if g == NG - 1:
                pass

            def body(b, _, g=g):
                step = g * B + b
                attn_step(step, g, b)
                if g == NG - 1:
                    @pl.when(step + NBUF == NSTEP)
                    def _():
                        for c in range(NW2):
                            w2_copy(c).start()
                return 0

            lax.fori_loop(0, B, body, 0)

            wo_copy(g).wait()
            acc = acc + jnp.dot(o_v[...].astype(dt), wo_v[pl.ds(g * GR, GR), :],
                                preferred_element_type=f32)
            if g == 1:
                w1_cp.wait()
                w3_cp.wait()
                gate = jnp.dot(xn, w1_v[...], preferred_element_type=f32).astype(dt).astype(f32)
                up = jnp.dot(xn, w3_v[...], preferred_element_type=f32).astype(dt).astype(f32)
                h = ((gate * jax.nn.sigmoid(gate)).astype(dt).astype(f32) * up).astype(dt)

        ffn = jnp.zeros((B, D), f32)
        for c in range(NW2):
            w2_copy(c).wait()
            ffn = ffn + jnp.dot(h[:, c * FC:(c + 1) * FC], w2_v[pl.ds(c * FC, FC), :],
                                preferred_element_type=f32)
        out_ref[...] = (x + acc + ffn).astype(out_ref.dtype)

    kt = jnp.swapaxes(A_k_cache, 2, 3).reshape(B * H * Dh, Sk)
    vt = jnp.swapaxes(A_v_cache, 2, 3).reshape(B * H * Dh, Sk)
    any_spec = pl.BlockSpec(memory_space=pl.ANY)
    out = pl.pallas_call(
        kernel_function,
        in_specs=[any_spec] * 8,
        out_specs=pl.BlockSpec(memory_space=pltpu.VMEM),
        out_shape=jax.ShapeDtypeStruct((B, D), dt),
        scratch_shapes=[
            pltpu.VMEM((B, D), dt),
            pltpu.VMEM(A_wq.shape, dt),
            pltpu.VMEM(A_wo.shape, dt),
            pltpu.VMEM(B_w1.shape, dt),
            pltpu.VMEM(B_w3.shape, dt),
            pltpu.VMEM(B_w2.shape, dt),
            pltpu.VMEM((NBUF, GR, W), dt),
            pltpu.VMEM((NBUF, GR, W), dt),
            pltpu.VMEM((B, H * Dh), f32),
            pltpu.VMEM((B, GR), f32),
            pltpu.SemaphoreType.DMA((4,)),
            pltpu.SemaphoreType.DMA((NG,)),
            pltpu.SemaphoreType.DMA((NW2,)),
            pltpu.SemaphoreType.DMA((NBUF,)),
            pltpu.SemaphoreType.DMA((NBUF,)),
        ],
        compiler_params=pltpu.CompilerParams(vmem_limit_bytes=100 * 1024 * 1024),
    )(A_x.reshape(B, D), kt, vt, A_wq, A_wo, B_w1, B_w3, B_w2)
    return out.reshape(B, Sq, D)
```

```python
import jax
import jax.numpy as jnp
from jax import lax
import jax.experimental.pallas as pl
import jax.experimental.pallas.tpu as pltpu

HG = 8
NBUF = 3
NW2 = 3
LN_EPS = 1e-5


@jax.jit
def pallas_parallel_sum__sliding_block_cached__glu_gated_swiglu__decode_kernel(
    A_x: jax.Array,
    A_k_cache: jax.Array,
    A_v_cache: jax.Array,
    A_wq: jax.Array,
    A_wo: jax.Array,
    B_x: jax.Array,
    B_w1: jax.Array,
    B_w3: jax.Array,
    B_w2: jax.Array,
):
    del B_x
    B, Sq, D = A_x.shape
    _, H, Sk, Dh = A_k_cache.shape
    F = B_w1.shape[1]
    assert Sq == 1 and B <= 8 and H % HG == 0 and A_wq.shape == (D, H * Dh)
    W = min(4096, max(256, Sk // 4))
    NG = H // HG
    GR = HG * Dh
    NSTEP = NG * B
    FC = F // NW2
    scale = Dh ** -0.5
    f32, bf16 = jnp.float32, jnp.bfloat16
    dt = A_x.dtype

    def kernel_function(x_hbm, kt_hbm, vt_hbm, wq_hbm, wo_hbm, w1_hbm, w3_hbm, w2_hbm,
                        out_ref,
                        x_v, wq_v, wo_v, w1_v, w3_v, w2_v, kbuf, vbuf, q_v, o_v,
                        sem_w, sem_wo, sem_w2, sem_k, sem_v):

        def kv_copy(src, dst, sem, step):
            g, b = step // B, step % B
            row = (b * NG + g) * GR
            slot = step % NBUF
            if not isinstance(step, int):
                row = pl.multiple_of(row, GR)
            return pltpu.make_async_copy(
                src.at[pl.ds(row, GR), pl.ds(Sk - W, W)], dst.at[slot], sem.at[slot])

        def k_copy(step):
            return kv_copy(kt_hbm, kbuf, sem_k, step)

        def v_copy(step):
            return kv_copy(vt_hbm, vbuf, sem_v, step)

        def wo_copy(g):
            return pltpu.make_async_copy(
                wo_hbm.at[pl.ds(g * GR, GR)], wo_v.at[pl.ds(g * GR, GR)], sem_wo.at[g])

        def w2_copy(c):
            return pltpu.make_async_copy(
                w2_hbm.at[pl.ds(c * FC, FC)], w2_v.at[pl.ds(c * FC, FC)], sem_w2.at[c])

        x_cp = pltpu.make_async_copy(x_hbm, x_v, sem_w.at[0])
        wq_cp = pltpu.make_async_copy(wq_hbm, wq_v, sem_w.at[1])
        w1_cp = pltpu.make_async_copy(w1_hbm, w1_v, sem_w.at[2])
        w3_cp = pltpu.make_async_copy(w3_hbm, w3_v, sem_w.at[3])

        wq_cp.start()
        x_cp.start()
        for s in range(NBUF):
            k_copy(s).start()
            v_copy(s).start()

        x_cp.wait()
        x = x_v[...].astype(f32)
        mean = jnp.mean(x, axis=-1, keepdims=True)
        xc = x - mean
        var = jnp.mean(xc * xc, axis=-1, keepdims=True)
        xn = (xc / jnp.sqrt(var + LN_EPS)).astype(dt)

        wq_cp.wait()
        q = jnp.dot(xn, wq_v[...], preferred_element_type=f32)
        q_v[...] = q.astype(dt).astype(f32)

        col = lax.broadcasted_iota(jnp.int32, (HG, GR), 1)
        lo = lax.broadcasted_iota(jnp.int32, (HG, GR), 0) * Dh
        diag = jnp.logical_and(col >= lo, col < lo + Dh)

        def tail_start(step):
            @pl.when(step == NSTEP - 2)
            def _():
                wo_copy(NG - 1).start()
                for c in range(NW2):
                    w2_copy(c).start()

        def attn_step(step, g, b):
            slot = step % NBUF
            qrow = q_v[pl.ds(b, 1), pl.ds(g * GR, GR)]
            qd = jnp.where(diag, jnp.broadcast_to(qrow, (HG, GR)), 0.0).astype(dt)
            k_copy(step).wait()
            s = jnp.dot(qd, kbuf[slot], preferred_element_type=f32) * scale

            @pl.when(step + NBUF < NSTEP)
            def _():
                k_copy(step + NBUF).start()

            m = jnp.max(s, axis=-1, keepdims=True)
            e = jnp.exp(s - m)
            p = (e / jnp.sum(e, axis=-1, keepdims=True)).astype(dt)
            v_copy(step).wait()
            if g == NG - 1:
                tail_start(step)
            o = lax.dot_general(p, vbuf[slot], (((1,), (1,)), ((), ())),
                                preferred_element_type=f32)

            @pl.when(step + NBUF < NSTEP)
            def _():
                v_copy(step + NBUF).start()

            o_v[pl.ds(b, 1), :] = jnp.sum(jnp.where(diag, o, 0.0), axis=0, keepdims=True)

        acc = jnp.zeros((B, D), f32)
        h = None
        for g in range(NG):
            if g < NG - 1:
                wo_copy(g).start()
            if g == 0:
                w1_cp.start()
            if g == 1:
                w3_cp.start()

            def body(b, _, g=g):
                step = g * B + b
                attn_step(step, g, b)
                return 0

            lax.fori_loop(0, B, body, 0)

            wo_copy(g).wait()
            acc = acc + jnp.dot(o_v[...].astype(dt), wo_v[pl.ds(g * GR, GR), :],
                                preferred_element_type=f32)
            if g == 1:
                w1_cp.wait()
                w3_cp.wait()
                gate = jnp.dot(xn, w1_v[...], preferred_element_type=f32).astype(dt).astype(f32)
                up = jnp.dot(xn, w3_v[...], preferred_element_type=f32).astype(dt).astype(f32)
                h = ((gate * jax.nn.sigmoid(gate)).astype(dt).astype(f32) * up)
                h = [h[:, c * FC:(c + 1) * FC].astype(dt) for c in range(NW2)]

        acc = x + acc
        for c in range(NW2):
            w2_copy(c).wait()
            acc = acc + jnp.dot(h[c], w2_v[pl.ds(c * FC, FC), :],
                                preferred_element_type=f32)
        out_ref[...] = acc.astype(out_ref.dtype)

    kt = jnp.swapaxes(A_k_cache, 2, 3).reshape(B * H * Dh, Sk)
    vt = jnp.swapaxes(A_v_cache, 2, 3).reshape(B * H * Dh, Sk)
    any_spec = pl.BlockSpec(memory_space=pl.ANY)
    out = pl.pallas_call(
        kernel_function,
        in_specs=[any_spec] * 8,
        out_specs=pl.BlockSpec(memory_space=pltpu.VMEM),
        out_shape=jax.ShapeDtypeStruct((B, D), dt),
        scratch_shapes=[
            pltpu.VMEM((B, D), dt),
            pltpu.VMEM(A_wq.shape, dt),
            pltpu.VMEM(A_wo.shape, dt),
            pltpu.VMEM(B_w1.shape, dt),
            pltpu.VMEM(B_w3.shape, dt),
            pltpu.VMEM(B_w2.shape, dt),
            pltpu.VMEM((NBUF, GR, W), dt),
            pltpu.VMEM((NBUF, GR, W), dt),
            pltpu.VMEM((B, H * Dh), f32),
            pltpu.VMEM((B, GR), f32),
            pltpu.SemaphoreType.DMA((4,)),
            pltpu.SemaphoreType.DMA((NG,)),
            pltpu.SemaphoreType.DMA((NW2,)),
            pltpu.SemaphoreType.DMA((NBUF,)),
            pltpu.SemaphoreType.DMA((NBUF,)),
        ],
        compiler_params=pltpu.CompilerParams(vmem_limit_bytes=100 * 1024 * 1024),
    )(A_x.reshape(B, D), kt, vt, A_wq, A_wo, B_w1, B_w3, B_w2)
    return out.reshape(B, Sq, D)
```
